```python
import jax
import jax.numpy as jnp

def _softmax(x, axis=-1):
    return jax.nn.softmax(x, axis=axis)
def _gelu(x):
    return jax.nn.gelu(x, approximate=True)
def _silu(x):
    return jax.nn.silu(x)
def _sigmoid(x):
    return jax.nn.sigmoid(x)
def _layernorm(x, axis=-1, eps=1e-5):
    m = jnp.mean(x, axis=axis, keepdims=True)
    v = jnp.var(x, axis=axis, keepdims=True)
    return (x - m) / jnp.sqrt(v + eps)
def _scatter_add(tgt, idx, src, axis=0):
    return tgt.at[idx].add(src)
def _segment_sum(src, seg, n):
    return jax.ops.segment_sum(src, seg, n)
class _Rng:
    def __init__(self, key):
        self._k = key
    def _next(self):
        self._k, sub = jax.random.split(self._k)
        return sub
    def normal(self, shape):
        return jax.random.normal(self._next(), shape, dtype=jnp.bfloat16)
    def randint(self, lo, hi, shape):
        return jax.random.randint(self._next(), shape, lo, hi, dtype=jnp.int32)
    def uniform(self, shape, lo=0.0, hi=1.0):
        return jax.random.uniform(self._next(), shape, jnp.bfloat16, lo, hi)
    def permutation(self, n):
        return jax.random.permutation(self._next(), n)


kernel_name = 'standalone__mha_softmax__near_ridge'

def _fwd_setup_inputs():
    _rng = _Rng(jax.random.key(int.from_bytes(__import__("os").urandom(4), "little")))
    _w = (lambda a: (lambda t: t.astype(jnp.bfloat16) if jnp.issubdtype(t.dtype, jnp.floating) else t)(jnp.asarray(a)))
    B, H, Sq, Sk, D = 16, 32, 384, 1024, 128
    return {
        "q": _w((lambda *s: _rng.normal(s) * 0.05)(B, H, Sq, D)),
        "k": _w((lambda *s: _rng.normal(s) * 0.05)(B, H, Sk, D)),
        "v": _w((lambda *s: _rng.normal(s) * 0.05)(B, H, Sk, D)),
    }

def _fwd_reference(q, k, v):
    scale = q.shape[-1] ** -0.5
    scores = jnp.einsum("bhqd,bhkd->bhqk", q, k) * scale
    p = _softmax(scores, axis=-1)
    return jnp.einsum("bhqk,bhkd->bhqd", p, v)


def setup_inputs():
    _inp = _fwd_setup_inputs()
    _gk = jax.random.fold_in(jax.random.key(int.from_bytes(__import__("os").urandom(4), "little")), 2**31 - 1)
    _shapes = [[16, 32, 384, 128]]
    _dtypes = ['bfloat16']
    _gks = jax.random.split(_gk, len(_shapes))
    _gs = [jax.random.normal(k, s, dtype=jnp.dtype(d)) * 0.05 for k, s, d in zip(_gks, _shapes, _dtypes)]
    _inp["grad_out"] = _gs[0]
    return _inp

def reference(q, k, v, grad_out):
    _const = dict()
    def _f(*_d):
        return _fwd_reference(**{'q': _d[0], 'k': _d[1], 'v': _d[2], **_const})
    _out, _vjp = jax.vjp(_f, q, k, v)
    _grads = _vjp(grad_out)
    _out0 = jnp.asarray(_out)
    return (_out0, *[jnp.asarray(_g) for _g in _grads])
```

```python
import functools, math
import jax, jax.numpy as jnp
from jax import lax
import jax.experimental.pallas as pl
import jax.experimental.pallas.tpu as pltpu
F32, BF16, U32 = jnp.float32, jnp.bfloat16, jnp.uint32
NT = (((1,), (1,)), ((), ()))
NN = (((1,), (0,)), ((), ()))
def dot(a, b, dn): return lax.dot_general(a, b, dn, preferred_element_type=F32)
def up(x): return pltpu.bitcast(x, BF16)
def dn(x): return pltpu.bitcast(x, U32)
def recip(l):
    r0 = pl.reciprocal(l, approx=True)
    return r0 * (2.0 - l * r0)

def build(hb=4, cp={}, order="ACDBFE", ns=1, first=None, last=None, lscr=True, foldc=False, pscr=True, late=False):
    def kernel(q_ref, k_ref, v_ref, do_ref, o_ref, dq_ref, dk_ref, dv_ref, *scr):
        Sq, D = q_ref.shape[1:]
        Sk = k_ref.shape[1]
        nt = Sk // 128
        hk, ht = Sk // 2, nt // 2
        z = pl.program_id(0) % 2
        scale = D ** -0.5
        c = scale * math.log2(math.e)
        npers = len(scr) // ns
        def ld(ref, h, p=None):
            rb = ref.bitcast(U32)
            return up(rb[h] if p is None else rb[h, p * hk // 2:(p + 1) * hk // 2, :])
        def ldw(ref, p):
            rb = ref.bitcast(U32)
            return up(jnp.concatenate([rb[z, j] for j in range(p * ht, (p + 1) * ht)], axis=1))
        def stw(ref, p, x):
            for j in range(ht):
                ref[z, p * ht + j] = x[:, j * 128:(j + 1) * 128].astype(BF16)
        def wide(x): return jnp.concatenate([x] * ht, axis=1)
        def bl(x): return jnp.broadcast_to(x, (x.shape[0], 128))
        def fold(op, x): return functools.reduce(op, [x[:, j * 128:(j + 1) * 128] for j in range(ht)])
        def ex(x): return jnp.exp2(x if foldc else x * c)
        def via(ref, p, x):
            if not lscr: return x
            ref[z, p] = dn(x)
            return up(ref[z, p])
        def stage(name, h):
            e_scr, ds_scr, m_scr, l_scr, a_scr, r_scr, dl_scr, p_scr, m2_scr, l2_scr, lo_scr, lq_scr = scr[(h % ns) * npers:(h % ns + 1) * npers]
            def two(lhs_scr, rhs_ref):
                x1 = dot(ldw(lhs_scr, 0), ld(rhs_ref, h, 0), NN)
                if pscr:
                    p_scr[z] = x1
                    x1 = p_scr[z]
                return x1 * a_scr[z] + dot(ldw(lhs_scr, 1), ld(rhs_ref, h, 1), NN)
            def twoT(x2, l_scr_, w_scr, out_ref):
                xs = [x2 * a_scr[z], x2]
                for p in range(2):
                    y = dot(via(l_scr_, p, xs[p].astype(BF16).T), ldw(w_scr, p), NN)
                    out_ref.bitcast(U32)[h, p * hk // 2:(p + 1) * hk // 2, :] = dn(y.astype(BF16).T)
            if name == "A":
                q = ld(q_ref, h)
                if foldc: q = (q.astype(F32) * c).astype(BF16)
                s = dot(q, ld(k_ref, h, 0), NT)
                m1 = bl(jnp.max(fold(jnp.maximum, s), axis=1, keepdims=True))
                e = ex(s - wide(m1))
                stw(e_scr, 0, e)
                m_scr[z] = m1
                l_scr[z] = fold(jnp.add, e)
                s = dot(q, ld(k_ref, h, 1), NT)
                m = bl(jnp.max(jnp.maximum(fold(jnp.maximum, s), m_scr[z]), axis=1, keepdims=True))
                e = ex(s - wide(m))
                stw(e_scr, 1, e)
                l2 = fold(jnp.add, e)
                if late:
                    m2_scr[z] = m
                    l2_scr[z] = l2
                else:
                    a = ex(m_scr[z] - m)
                    a_scr[z] = a
                    r_scr[z] = bl(recip(jnp.sum(l_scr[z] * a + l2, axis=1, keepdims=True)))
            elif name == "B":
                for p in range(2):
                    dp = dot(ld(do_ref, h), ld(v_ref, h, p), NT)
                    stw(ds_scr, p, ldw(e_scr, p).astype(F32) * (dp - wide(dl_scr[z])))
            elif name == "C":
                o = two(e_scr, v_ref) * r_scr[z]
                dl_scr[z] = bl(jnp.sum(ld(do_ref, h).astype(F32) * o, axis=1, keepdims=True))
                o_ref[h] = o.astype(BF16)
            elif name == "D":
                twoT(ld(do_ref, h).astype(F32) * r_scr[z], lo_scr, e_scr, dv_ref)
            elif name == "E":
                dq_ref[h] = (two(ds_scr, k_ref) * (r_scr[z] * scale)).astype(BF16)
            elif name == "F":
                twoT(ld(q_ref, h).astype(F32) * (r_scr[z] * scale), lq_scr, ds_scr, dk_ref)
        if first is None:
            for n in order:
                if n.islower(): stage(n.upper(), 0)
        for h in range(hb):
            od = first if (h == 0 and first) else (last if (h == hb - 1 and last) else order)
            for n in od:
                if n.islower():
                    if h + 1 < hb: stage(n.upper(), h + 1)
                else: stage(n, h)

    @jax.jit
    def f(q, k, v, grad_out):
        B, H, Sq, D = q.shape; Sk = k.shape[2]; N = B * H
        r = lambda x: x.reshape(N, x.shape[2], D)
        sq = pl.BlockSpec((hb, Sq, D), lambda i: (i, 0, 0)); sk = pl.BlockSpec((hb, Sk, D), lambda i: (i, 0, 0))
        oq = jax.ShapeDtypeStruct((N, Sq, D), q.dtype); ok = jax.ShapeDtypeStruct((N, Sk, D), q.dtype)
        V = pltpu.VMEM
        per = [V((2, Sk // 128, Sq, 128), BF16)] * 2 + [V((2, Sq, 128), F32)] * 8 + [V((2, 2, D // 2, Sq), U32)] * 2
        o, dq, dk, dv = pl.pallas_call(kernel, grid=(N // hb,), in_specs=[sq, sk, sk, sq], out_specs=[sq, sq, sk, sk],
            out_shape=[oq, oq, ok, ok], name="mha", scratch_shapes=per * ns,
            compiler_params=pltpu.CompilerParams(dimension_semantics=("parallel",), vmem_limit_bytes=100 * 2**20, **cp))(r(q), r(k), r(v), r(grad_out))
        return o.reshape(q.shape), dq.reshape(q.shape), dk.reshape(k.shape), dv.reshape(k.shape)
    return f


pallas_standalone__mha_softmax__near_ridge_kernel = build()
```

```python
import functools
import math

import jax
import jax.numpy as jnp
from jax import lax
from jax.experimental import pallas as pl
from jax.experimental.pallas import tpu as pltpu

F32, BF16, U32 = jnp.float32, jnp.bfloat16, jnp.uint32
NT = (((1,), (1,)), ((), ()))
NN = (((1,), (0,)), ((), ()))


def _dot(a, b, dims):
    return lax.dot_general(a, b, dims, preferred_element_type=F32)


def _bf(x):
    return pltpu.bitcast(x, BF16)


def _u32(x):
    return pltpu.bitcast(x, U32)


def _recip(l):
    r0 = pl.reciprocal(l, approx=True)
    return r0 * (2.0 - l * r0)


def _kernel(q_hbm, k_hbm, v_hbm, do_hbm, o_hbm, dq_hbm, dk_hbm, dv_hbm,
            qd, kv, oq, gkv, isem, osem,
            e_scr, ds_scr, m1_scr, l1_scr, m2_scr, l2_scr, a_scr, r_scr, dl_scr, p_scr, lo_scr, lq_scr,
            *, hb, nr, dly, top):
    n_groups = (q_hbm.shape[0] - nr) // hb
    d = qd.shape[2]
    hk = kv.shape[1] // 2
    ht = hk // 128
    scale = d ** -0.5
    c = scale * math.log2(math.e)
    ins = ((k_hbm, kv, 0, 0), (q_hbm, qd, 0, 1), (v_hbm, kv, 1, 0), (do_hbm, qd, 1, 1))
    outs = ((o_hbm, oq, 0, 1), (dv_hbm, gkv, 1, 0), (dk_hbm, gkv, 0, 0), (dq_hbm, oq, 1, 1))

    def copy_in(g, n, s, sem):
        return [pltpu.make_async_copy(hbm.at[pl.ds(g, n)], buf.at[pl.ds(s[w], n)], isem.at[sem + t])
                for hbm, buf, w, t in ins]

    def copy_out(g, n, s, sem, which):
        return [pltpu.make_async_copy(buf.at[pl.ds(s[w], n)], hbm.at[pl.ds(g, n)], osem.at[sem + t])
                for hbm, buf, w, t in (outs[u] for u in which)]

    def start(copies):
        for cp in copies:
            cp.start()

    def wait_all(bufs, s0, n, sems, sem):
        for t, buf in enumerate(bufs):
            view = buf.at[pl.ds(s0, n)]
            pltpu.make_async_copy(view, view, sems.at[sem + t]).wait()

    def head(s, z, zero, emit, mid=None):
        zu = zero.astype(U32)

        def ld(ref, w, p=None):
            rb = ref.bitcast(U32)
            return _bf(rb[s[w]] if p is None else rb[s[w], p * hk // 2:(p + 1) * hk // 2, :])

        def ldw(ref, p):
            rb = ref.bitcast(U32)
            return _bf(jnp.concatenate([rb[z, j] for j in range(p * ht, (p + 1) * ht)], axis=1))

        def stw(ref, p, x):
            for j in range(ht):
                ref[z, p * ht + j] = x[:, j * 128:(j + 1) * 128].astype(BF16)

        def wide(x):
            return jnp.concatenate([x] * ht, axis=1)

        def lanes(x):
            return jnp.broadcast_to(x, (x.shape[0], 128))

        def fold(op, x):
            return functools.reduce(op, [x[:, j * 128:(j + 1) * 128] for j in range(ht)])

        def grad_kv(x, lhs_scr, w_scr, w):
            for p, xp in enumerate((x * a_scr[z], x)):
                lhs_scr[z, p] = _u32(xp.astype(BF16).T)
                y = _dot(_bf(lhs_scr[z, p]), ldw(w_scr, p), NN)
                gkv.bitcast(U32)[s[w], p * hk // 2:(p + 1) * hk // 2, :] = _u32(y.astype(BF16).T)

        q = ld(qd, 0)
        sc = _dot(q, ld(kv, 0, 0), NT)
        m1 = lanes(jnp.max(fold(jnp.maximum, sc), axis=1, keepdims=True))
        e = jnp.exp2((sc - wide(m1)) * c)
        stw(e_scr, 0, e)
        m1_scr[z] = m1
        l1_scr[z] = fold(jnp.add, e)
        sc = _dot(q, ld(kv, 0, 1), NT)
        m = lanes(jnp.max(jnp.maximum(fold(jnp.maximum, sc), m1_scr[z]), axis=1, keepdims=True))
        e = jnp.exp2((sc - wide(m)) * c)
        stw(e_scr, 1, e)
        m2_scr[z] = m
        l2_scr[z] = fold(jnp.add, e)
        if mid is not None:
            mid()
        x1 = _dot(ldw(e_scr, 0), ld(kv, 1, 0), NN)
        if dly is not None:
            vb = kv.bitcast(U32)
            vb[s[1] + zero, 0:8, :] = vb[s[1], 0:8, :] | (_u32(x1[dly:dly + 8]) & zu)
        m1 = pltpu.bitcast(_u32(m1_scr[z]) | (_u32(x1) & zu), F32)
        a = jnp.exp2((m1 - m2_scr[z]) * c)
        a_scr[z] = a
        p_scr[z] = x1 * a
        r_scr[z] = lanes(_recip(jnp.sum(l1_scr[z] * a + l2_scr[z], axis=1, keepdims=True)))
        o = (p_scr[z] + _dot(ldw(e_scr, 1), ld(kv, 1, 1), NN)) * r_scr[z]
        dl_scr[z] = lanes(jnp.sum(ld(qd, 1).astype(F32) * o, axis=1, keepdims=True))
        oq[s[0]] = o.astype(BF16)
        emit((0,))
        grad_kv(ld(qd, 1).astype(F32) * r_scr[z], lo_scr, e_scr, 1)
        for p in range(2):
            dp = _dot(ld(qd, 1), ld(kv, 1, p), NT)
            stw(ds_scr, p, ldw(e_scr, p).astype(F32) * (dp - wide(dl_scr[z])))
        grad_kv(ld(qd, 0).astype(F32) * (r_scr[z] * scale), lq_scr, ds_scr, 0)
        p_scr[z] = _dot(ldw(ds_scr, 0), ld(kv, 0, 0), NN)
        k2 = _u32(ld(kv, 0, 1))
        k2 = jnp.concatenate([k2[:8] | (gkv.bitcast(U32)[s[0] + zero, 0:8, :] & zu), k2[8:]], axis=0)
        dq = p_scr[z] * a_scr[z] + _dot(ldw(ds_scr, 1), _bf(k2), NN)
        oq[s[1]] = (dq * (r_scr[z] * scale)).astype(BF16)
        emit((1, 2, 3))

    def ramp_slots(j):
        return 4 * hb + j, 4 * hb + nr + j

    ahead = -(-(nr + hb - 1) // max(nr - 1, 1))
    start(copy_in(0, 1, ramp_slots(0), 2))

    def ramp(j, carry):
        for cp in copy_in(j, 1, ramp_slots(j), 2 + 2 * j):
            cp.wait()

        def fetch(n):
            g = jnp.minimum(n, nr + hb - 1)
            early = g < nr
            s = (jnp.where(early, 4 * hb + g, g - nr), jnp.where(early, 4 * hb + nr + g, g - nr + hb))
            start(copy_in(g, 1, s, jnp.where(early, 2 + 2 * g, 0)))

        def prefetch(lo, hi):
            for u in range(lo, hi):
                n = 1 + ahead * j + u
                pl.when(n < nr + hb)(functools.partial(fetch, n))

        prefetch(0, top)
        head(ramp_slots(j), j & 1, lax.shift_right_logical(j, 20), lambda which: None,
             functools.partial(prefetch, top, ahead))
        return carry

    lax.fori_loop(0, nr, ramp, 0)
    start(copy_out(0, nr, ramp_slots(0), 4, range(4)))

    def group(i, carry):
        z = i & 1
        s0 = z * (2 * hb)
        wait_all((kv, qd), s0, 2 * hb, isem, 0)
        pl.when(i > 1)(lambda: wait_all((gkv, oq), s0, 2 * hb, osem, 2 * z))
        zero = lax.shift_right_logical(i, 20)
        for j in range(hb):
            s = (s0 + j, s0 + hb + j)
            g = nr + i * hb + j
            head(s, z, zero, lambda which: start(copy_out(g, 1, s, 2 * z, which)))
            if j == 0:
                @pl.when(i + 1 < n_groups)
                def _():
                    s1 = 2 * hb - s0
                    start(copy_in(nr + jnp.minimum(i + 1, n_groups - 1) * hb, hb, (s1, s1 + hb), 0))
        return carry

    lax.fori_loop(0, n_groups, group, 0)
    wait_all((gkv, oq), 4 * hb, 2 * nr, osem, 4)
    for z in (n_groups % 2, 1 - n_groups % 2):
        wait_all((gkv, oq), z * 2 * hb, 2 * hb, osem, 2 * z)


def build(hb=14, nr=8, dly=128, top=0):
    @jax.jit
    def mha(q, k, v, grad_out):
        b, h, sq, d = q.shape
        sk, n = k.shape[2], b * h
        assert (n - nr) % hb == 0 and (n - nr) // hb >= 2 and d == 128 and sk % 256 == 0
        flat = lambda x: x.reshape(n, x.shape[2], d)
        spec = pl.BlockSpec(memory_space=pl.ANY)
        out_q = jax.ShapeDtypeStruct((n, sq, d), q.dtype)
        out_k = jax.ShapeDtypeStruct((n, sk, d), q.dtype)
        slots = 4 * hb + 2 * nr
        buf_q, buf_k = pltpu.VMEM((slots, sq, d), BF16), pltpu.VMEM((slots, sk, d), BF16)
        scratch = [buf_q, buf_k, buf_q, buf_k,
                   pltpu.SemaphoreType.DMA((2 + 2 * nr,)), pltpu.SemaphoreType.DMA((6,))]
        scratch += [pltpu.VMEM((2, sk // 128, sq, 128), BF16)] * 2
        scratch += [pltpu.VMEM((2, sq, 128), F32)] * 8
        scratch += [pltpu.VMEM((2, 2, d // 2, sq), U32)] * 2
        o, dq, dk, dv = pl.pallas_call(
            functools.partial(_kernel, hb=hb, nr=nr, dly=dly, top=top),
            in_specs=[spec] * 4, out_specs=[spec] * 4, out_shape=[out_q, out_q, out_k, out_k],
            scratch_shapes=scratch, name="mha",
            compiler_params=pltpu.CompilerParams(vmem_limit_bytes=100 * 2 ** 20, disable_bounds_checks=True),
        )(flat(q), flat(k), flat(v), flat(grad_out))
        return o.reshape(q.shape), dq.reshape(q.shape), dk.reshape(k.shape), dv.reshape(k.shape)
    return mha


pallas_standalone__mha_softmax__near_ridge_kernel = build()
```

```python
import functools
import math

import jax
import jax.numpy as jnp
from jax import lax
from jax.experimental import pallas as pl
from jax.experimental.pallas import tpu as pltpu

F32, BF16, U32 = jnp.float32, jnp.bfloat16, jnp.uint32
NT = (((1,), (1,)), ((), ()))
NN = (((1,), (0,)), ((), ()))


def _dot(a, b, dims):
    return lax.dot_general(a, b, dims, preferred_element_type=F32)


def _bf(x):
    return pltpu.bitcast(x, BF16)


def _u32(x):
    return pltpu.bitcast(x, U32)


def _recip(l):
    r0 = pl.reciprocal(l, approx=True)
    return r0 * (2.0 - l * r0)


def _kernel(q_hbm, k_hbm, v_hbm, do_hbm, o_hbm, dq_hbm, dk_hbm, dv_hbm,
            qd, kv, oq, gkv, isem, osem,
            e_scr, ds_scr, m1_scr, l1_scr, m2_scr, l2_scr, a_scr, r_scr, dl_scr, p_scr, lo_scr, lq_scr,
            *, hb, nr, dly):
    n_groups = (q_hbm.shape[0] - nr) // hb
    d = qd.shape[2]
    hk = kv.shape[1] // 2
    ht = hk // 128
    scale = d ** -0.5
    c = scale * math.log2(math.e)
    ins = ((k_hbm, kv, 0, 0), (q_hbm, qd, 0, 1), (v_hbm, kv, 1, 0), (do_hbm, qd, 1, 1))
    outs = ((o_hbm, oq, 0, 0), (dv_hbm, gkv, 1, 1), (dk_hbm, gkv, 0, 2), (dq_hbm, oq, 1, 3))

    def copy_in(g, n, s, sem):
        return [pltpu.make_async_copy(hbm.at[pl.ds(g, n)], buf.at[pl.ds(s[w], n)], isem.at[sem + t])
                for hbm, buf, w, t in ins]

    def copy_out(g, n, s, sem, which=(0, 1, 2, 3)):
        return [pltpu.make_async_copy(buf.at[pl.ds(s[w], n)], hbm.at[pl.ds(g, n)], osem.at[sem + t])
                for hbm, buf, w, t in (outs[u] for u in which)]

    def start(copies):
        for cp in copies:
            cp.start()

    def wait(copies):
        for cp in copies:
            cp.wait()

    def wait_group_out(i, z):
        wait(copy_out(nr + i * hb, hb, (z * (2 * hb), z * (2 * hb) + hb), 4 * z))

    def head(s, z, zero, emit, mid=None):
        zu = zero.astype(U32)

        def ld(ref, w, p=None):
            rb = ref.bitcast(U32)
            return _bf(rb[s[w]] if p is None else rb[s[w], p * hk // 2:(p + 1) * hk // 2, :])

        def ldw(ref, p):
            rb = ref.bitcast(U32)
            return _bf(jnp.concatenate([rb[z, j] for j in range(p * ht, (p + 1) * ht)], axis=1))

        def stw(ref, p, x):
            for j in range(ht):
                ref[z, p * ht + j] = x[:, j * 128:(j + 1) * 128].astype(BF16)

        def wide(x):
            return jnp.concatenate([x] * ht, axis=1)

        def lanes(x):
            return jnp.broadcast_to(x, (x.shape[0], 128))

        def fold(op, x):
            return functools.reduce(op, [x[:, j * 128:(j + 1) * 128] for j in range(ht)])

        def grad_kv(x, lhs_scr, w_scr, w):
            for p, xp in enumerate((x * a_scr[z], x)):
                lhs_scr[z, p] = _u32(xp.astype(BF16).T)
                y = _dot(_bf(lhs_scr[z, p]), ldw(w_scr, p), NN)
                gkv.bitcast(U32)[s[w], p * hk // 2:(p + 1) * hk // 2, :] = _u32(y.astype(BF16).T)

        q = ld(qd, 0)
        sc = _dot(q, ld(kv, 0, 0), NT)
        m1 = lanes(jnp.max(fold(jnp.maximum, sc), axis=1, keepdims=True))
        e = jnp.exp2((sc - wide(m1)) * c)
        stw(e_scr, 0, e)
        m1_scr[z] = m1
        l1_scr[z] = fold(jnp.add, e)
        sc = _dot(q, ld(kv, 0, 1), NT)
        m = lanes(jnp.max(jnp.maximum(fold(jnp.maximum, sc), m1_scr[z]), axis=1, keepdims=True))
        e = jnp.exp2((sc - wide(m)) * c)
        stw(e_scr, 1, e)
        m2_scr[z] = m
        l2_scr[z] = fold(jnp.add, e)
        if mid is not None:
            mid()
        x1 = _dot(ldw(e_scr, 0), ld(kv, 1, 0), NN)
        vb = kv.bitcast(U32)
        vb[s[1] + zero, 0:8, :] = vb[s[1], 0:8, :] | (_u32(x1[dly:dly + 8]) & zu)
        m1 = pltpu.bitcast(_u32(m1_scr[z]) | (_u32(x1) & zu), F32)
        a = jnp.exp2((m1 - m2_scr[z]) * c)
        a_scr[z] = a
        p_scr[z] = x1 * a
        r_scr[z] = lanes(_recip(jnp.sum(l1_scr[z] * a + l2_scr[z], axis=1, keepdims=True)))
        o = (p_scr[z] + _dot(ldw(e_scr, 1), ld(kv, 1, 1), NN)) * r_scr[z]
        dl_scr[z] = lanes(jnp.sum(ld(qd, 1).astype(F32) * o, axis=1, keepdims=True))
        oq[s[0]] = o.astype(BF16)
        emit((0,))
        grad_kv(ld(qd, 1).astype(F32) * r_scr[z], lo_scr, e_scr, 1)
        for p in range(2):
            dp = _dot(ld(qd, 1), ld(kv, 1, p), NT)
            stw(ds_scr, p, ldw(e_scr, p).astype(F32) * (dp - wide(dl_scr[z])))
        grad_kv(ld(qd, 0).astype(F32) * (r_scr[z] * scale), lq_scr, ds_scr, 0)
        p_scr[z] = _dot(ldw(ds_scr, 0), ld(kv, 0, 0), NN)
        k2 = _u32(ld(kv, 0, 1))
        k2 = jnp.concatenate([k2[:8] | (gkv.bitcast(U32)[s[0] + zero, 0:8, :] & zu), k2[8:]], axis=0)
        dq = p_scr[z] * a_scr[z] + _dot(ldw(ds_scr, 1), _bf(k2), NN)
        oq[s[1]] = (dq * (r_scr[z] * scale)).astype(BF16)
        emit((1, 2, 3))

    def ramp_slots(j):
        return 4 * hb + j, 4 * hb + nr + j

    ahead = -(-(nr + hb - 1) // max(nr - 1, 1))
    start(copy_in(0, 1, ramp_slots(0), 2))

    def ramp(j, carry):
        wait(copy_in(j, 1, ramp_slots(j), 2 + 2 * j))

        def fetch(n):
            g = jnp.minimum(n, nr + hb - 1)
            early, lo, hi = g < nr, jnp.minimum(g, nr - 1), jnp.maximum(g - nr, 0)
            s = (jnp.where(early, 4 * hb + lo, hi), jnp.where(early, 4 * hb + nr + lo, hb + hi))
            start(copy_in(g, 1, s, jnp.where(early, 2 + 2 * lo, 0)))

        def prefetch():
            for u in range(ahead):
                n = 1 + ahead * j + u
                pl.when(n < nr + hb)(functools.partial(fetch, n))

        head(ramp_slots(j), j & 1, lax.shift_right_logical(j, 20), lambda which: None, prefetch)
        return carry

    lax.fori_loop(0, nr, ramp, 0)
    start(copy_out(0, nr, ramp_slots(0), 8))

    def group(i, carry):
        z = i & 1
        s0 = z * (2 * hb)
        for t, buf in enumerate((kv, qd)):
            view = buf.at[pl.ds(s0, 2 * hb)]
            pltpu.make_async_copy(view, view, isem.at[t]).wait()
        pl.when(i > 1)(lambda: wait_group_out(jnp.maximum(i - 2, 0), z))
        zero = lax.shift_right_logical(i, 20)
        for j in range(hb):
            s = (s0 + j, s0 + hb + j)
            g = nr + i * hb + j
            head(s, z, zero, lambda which: start(copy_out(g, 1, s, 4 * z, which)))
            if j == hb // 6:
                @pl.when(i + 1 < n_groups)
                def _():
                    s1 = 2 * hb - s0
                    start(copy_in(nr + jnp.minimum(i + 1, n_groups - 1) * hb, hb, (s1, s1 + hb), 0))
        return carry

    lax.fori_loop(0, n_groups, group, 0)
    wait(copy_out(0, nr, ramp_slots(0), 8))
    for i in (n_groups - 2, n_groups - 1):
        wait_group_out(i, i % 2)


def _build(hb=14, nr=8, dly=112):
    @jax.jit
    def mha(q, k, v, grad_out):
        b, h, sq, d = q.shape
        sk, n = k.shape[2], b * h
        assert (n - nr) % hb == 0 and (n - nr) // hb >= 2 and d == 128 and sk % 256 == 0
        flat = lambda x: x.reshape(n, x.shape[2], d)
        spec = pl.BlockSpec(memory_space=pl.ANY)
        out_q = jax.ShapeDtypeStruct((n, sq, d), q.dtype)
        out_k = jax.ShapeDtypeStruct((n, sk, d), q.dtype)
        slots = 4 * hb + 2 * nr
        buf_q, buf_k = pltpu.VMEM((slots, sq, d), BF16), pltpu.VMEM((slots, sk, d), BF16)
        scratch = [buf_q, buf_k, buf_q, buf_k,
                   pltpu.SemaphoreType.DMA((2 + 2 * nr,)), pltpu.SemaphoreType.DMA((12,))]
        scratch += [pltpu.VMEM((2, sk // 128, sq, 128), BF16)] * 2
        scratch += [pltpu.VMEM((2, sq, 128), F32)] * 8
        scratch += [pltpu.VMEM((2, 2, d // 2, sq), U32)] * 2
        o, dq, dk, dv = pl.pallas_call(
            functools.partial(_kernel, hb=hb, nr=nr, dly=dly),
            in_specs=[spec] * 4, out_specs=[spec] * 4, out_shape=[out_q, out_q, out_k, out_k],
            scratch_shapes=scratch, name="mha",
            compiler_params=pltpu.CompilerParams(vmem_limit_bytes=100 * 2 ** 20, disable_bounds_checks=True),
        )(flat(q), flat(k), flat(v), flat(grad_out))
        return o.reshape(q.shape), dq.reshape(q.shape), dk.reshape(k.shape), dv.reshape(k.shape)
    return mha


pallas_standalone__mha_softmax__near_ridge_kernel = _build()
```
